```python
import jax
import jax.numpy as jnp

def _softmax(x, axis=-1):
    return jax.nn.softmax(x, axis=axis)
def _gelu(x):
    return jax.nn.gelu(x, approximate=True)
def _silu(x):
    return jax.nn.silu(x)
def _sigmoid(x):
    return jax.nn.sigmoid(x)
def _layernorm(x, axis=-1, eps=1e-5):
    m = jnp.mean(x, axis=axis, keepdims=True)
    v = jnp.var(x, axis=axis, keepdims=True)
    return (x - m) / jnp.sqrt(v + eps)
def _scatter_add(tgt, idx, src, axis=0):
    return tgt.at[idx].add(src)
def _segment_sum(src, seg, n):
    return jax.ops.segment_sum(src, seg, n)
class _Rng:
    def __init__(self, key):
        self._k = key
    def _next(self):
        self._k, sub = jax.random.split(self._k)
        return sub
    def normal(self, shape):
        return jax.random.normal(self._next(), shape, dtype=jnp.bfloat16)
    def randint(self, lo, hi, shape):
        return jax.random.randint(self._next(), shape, lo, hi, dtype=jnp.int32)
    def uniform(self, shape, lo=0.0, hi=1.0):
        return jax.random.uniform(self._next(), shape, jnp.bfloat16, lo, hi)
    def permutation(self, n):
        return jax.random.permutation(self._next(), n)


kernel_name = 'concat_heads__ssm_conv_h3__softmax_full_mha__prompt'

def _fwd_setup_inputs():
    _rng = _Rng(jax.random.key(int.from_bytes(__import__("os").urandom(4), "little")))
    _w = (lambda a: (lambda t: t.astype(jnp.bfloat16) if jnp.issubdtype(t.dtype, jnp.floating) else t)(jnp.asarray(a)))
    def _A_setup():
        B, S, D = 1, 2048, 640
        ks = 4
        return {
            "q": _w((lambda *s: _rng.normal(s) * 0.05)(B, S, D)),
            "k": _w((lambda *s: _rng.normal(s) * 0.05)(B, S, D)),
            "v": _w((lambda *s: _rng.normal(s) * 0.05)(B, S, D)),
            "shift_k": _w((lambda *s: _rng.normal(s) * 0.05)(D, ks) * 0.5),
            "ssm_k": _w((lambda *s: _rng.normal(s) * 0.05)(D, S) * (1.0 / S ** 0.5)),
            "ssm_D": _w((lambda *s: _rng.normal(s) * 0.05)(D)),
        }
    _A_in = _A_setup()

    def _B_setup():
        B, S, D = 1, 2048, 640
        return {
            "x": _w((lambda *s: _rng.normal(s) * 0.05)(B, S, D)),
            "wqkv": _w((lambda *s: _rng.normal(s) * 0.05)(D, 3 * D)),
            "wo": _w((lambda *s: _rng.normal(s) * 0.05)(D, D)),
        }
    _B_in = _B_setup()

    return {
        "A_q": _A_in["q"],
        "A_k": _A_in["k"],
        "A_v": _A_in["v"],
        "A_shift_k": _A_in["shift_k"],
        "A_ssm_k": _A_in["ssm_k"],
        "A_ssm_D": _A_in["ssm_D"],
        "B_x": _B_in["x"],
        "B_wqkv": _B_in["wqkv"],
        "B_wo": _B_in["wo"],
    }

def _fwd_reference(A_q, A_k, A_v, A_shift_k, A_ssm_k, A_ssm_D, B_x, B_wqkv, B_wo):
    def _A_ref(q, k, v, shift_k, ssm_k, ssm_D):
        B, S, D = q.shape
        ks = shift_k.shape[-1]
        k_pad = jnp.pad(k, ((0, 0), (ks - 1, 0), (0, 0)))
        k_shift = jnp.zeros_like(k)
        for t in range(ks):
            k_shift = k_shift + k_pad[:, t:t + S, :] * shift_k[:, ks - 1 - t][None, None, :]
        kv = k_shift * v
        L = 2 * S
        kv_pad = jnp.pad(kv, ((0, 0), (0, S), (0, 0)))
        kf_pad = jnp.pad(ssm_k, ((0, 0), (0, S)))
        kv_f = (lambda x, axes=(-2,-1): jnp.fft.rfft2(x.astype(jnp.float32), axes=axes))(kv_pad[:, None, :, :], axes=(1, 2))
        kf_f = (lambda x, axes=(-2,-1): jnp.fft.rfft2(x.astype(jnp.float32), axes=axes))(kf_pad[:, None, :], axes=(1, 2))
        kf_f = (lambda x, *d: x.transpose(*d))(kf_f, 1, 2, 0)
        y_f = kv_f * kf_f[None, :, :, :]
        y = (lambda x, s, axes=(-2,-1): jnp.fft.irfft2(x, s=s, axes=axes).astype(jnp.bfloat16))(y_f, (1, L), axes=(1, 2))[:, 0, :S, :]
        y = y + kv * ssm_D[None, None, :]
        return q * y

    def _B_ref(x, wqkv, wo):
        B, S, D = x.shape
        H = 32; Dh = D // H
        qkv = (lambda x, *d: x.transpose(*d))((x @ wqkv).reshape(B, S, 3, H, Dh), 2, 0, 3, 1, 4)
        q, k, v = qkv[0], qkv[1], qkv[2]
        scale = Dh ** -0.5
        scores = jnp.einsum("bhqd,bhkd->bhqk", q, k) * scale
        p = _softmax(scores, axis=-1)
        o = jnp.einsum("bhqk,bhkd->bhqd", p, v)
        return (lambda x, *d: x.transpose(*d))(o, 0, 2, 1, 3).reshape(B, S, D) @ wo

    a = _A_ref(A_q, A_k, A_v, A_shift_k, A_ssm_k, A_ssm_D)
    b = _B_ref(B_x, B_wqkv, B_wo)
    return jnp.concatenate([a, b], axis=-1)


def setup_inputs():
    _inp = _fwd_setup_inputs()
    _gk = jax.random.fold_in(jax.random.key(int.from_bytes(__import__("os").urandom(4), "little")), 2**31 - 1)
    _shapes = [[1, 2048, 1280]]
    _dtypes = ['bfloat16']
    _gks = jax.random.split(_gk, len(_shapes))
    _gs = [jax.random.normal(k, s, dtype=jnp.dtype(d)) * 0.05 for k, s, d in zip(_gks, _shapes, _dtypes)]
    _inp["grad_out"] = _gs[0]
    return _inp

def reference(A_q, A_k, A_v, A_shift_k, A_ssm_k, A_ssm_D, B_x, B_wqkv, B_wo, grad_out):
    _const = dict()
    def _f(*_d):
        return _fwd_reference(**{'A_q': _d[0], 'A_k': _d[1], 'A_v': _d[2], 'A_shift_k': _d[3], 'A_ssm_k': _d[4], 'A_ssm_D': _d[5], 'B_x': _d[6], 'B_wqkv': _d[7], 'B_wo': _d[8], **_const})
    _out, _vjp = jax.vjp(_f, A_q, A_k, A_v, A_shift_k, A_ssm_k, A_ssm_D, B_x, B_wqkv, B_wo)
    _grads = _vjp(grad_out)
    _out0 = jnp.asarray(_out)
    return (_out0, *[jnp.asarray(_g) for _g in _grads])
```

```python
import math

import numpy as np
import jax
import jax.numpy as jnp
from jax import lax
import jax.experimental.pallas as pl
import jax.experimental.pallas.tpu as pltpu

S = 2048
D = 640
H = 32
DH = 20
KS = 4
TQ = 512
CK = 128
R = 24
NQ = S // TQ
NC = S // CK
NU = H * NQ
NG = H // 4
BL = 128
NB = S // BL
NCG = D // 128

OFF_O = 18
OFF_E = 19
OFF_A = 36
UNR = 2
S0 = 1
NIT = (NU * NC - OFF_A - S0) // (UNR * NC)

f32 = jnp.float32
bf16 = jnp.bfloat16
u32 = jnp.uint32
NN = (((1,), (0,)), ((), ()))
NT = (((1,), (1,)), ((), ()))

SCALE = float(DH) ** -0.5
LOG2E = math.log2(math.e)


def _dot(a, b, dims):
    return lax.dot_general(a, b, dims, preferred_element_type=f32)


def _up(x):
    return pltpu.bitcast(x, bf16)


def _pk(x):
    return pltpu.bitcast(x, u32)


def _rnd(x):
    return x.astype(bf16).astype(f32)


def _dft_mats():
    f = np.arange(BL, dtype=np.float64)[:, None] + 0.5
    n = np.arange(BL, dtype=np.float64)[None, :]
    th = 2.0 * np.pi * f * n / (2 * BL)
    fwd = np.concatenate([np.cos(th), -np.sin(th)], axis=0)
    inv = fwd.T / BL
    return fwd.astype(np.float32), inv.astype(np.float32)


def _kernel(q_hbm, k_hbm, v_hbm, sk_ref, ssmk_hbm, ssmd_ref, x_hbm, wqkv_hbm, wo_hbm, g_hbm,
            fw_ref, iv_ref,
            out_hbm, dq_hbm, dk_hbm, dv_hbm, dsk_ref, dssmk_hbm, dssmd_ref, dx_hbm, dwqkv_hbm,
            dwo_hbm,
            q_buf, k_buf, v_buf, h_buf, x_buf, w_buf, wo_buf, g_buf,
            qkvt, dot, vta, kwin, vwin, sems):
    in_pairs = [(wqkv_hbm, w_buf), (x_hbm, x_buf), (wo_hbm, wo_buf), (g_hbm, g_buf),
                (k_hbm, k_buf), (v_hbm, v_buf), (q_hbm, q_buf), (ssmk_hbm, h_buf)]
    in_cp = [pltpu.make_async_copy(s, d, sems.at[i]) for i, (s, d) in enumerate(in_pairs)]
    for c in in_cp:
        c.start()
    cp_w, cp_x, cp_wo, cp_g, cp_k, cp_v, cp_q, cp_h = in_cp

    def proj_phase(wt):
        cp_w.wait()
        for j in range(3 * D // 128):
            wt[j * 64:(j + 1) * 64, :] = _pk(w_buf[:, j * 128:(j + 1) * 128].T)
        cp_x.wait()

        def proj(i, c):
            part = i // NQ
            sb = i % NQ
            w = _up(wt[pl.ds(pl.multiple_of(part * (D // 2), 8), D // 2), :])
            xb = x_buf[pl.ds(pl.multiple_of(sb * TQ, TQ), TQ), :]
            r = _dot(w, xb, NT)
            r = r * jnp.where(part == 0, SCALE * LOG2E, 1.0)
            qkvt[pl.ds(pl.multiple_of(part * D, 8), D), pl.ds(pl.multiple_of(sb * TQ, TQ), TQ)] = _rnd(r)
            return c
        lax.fori_loop(0, 3 * NQ, proj, 0)

    pl.run_scoped(proj_phase, pltpu.VMEM((3 * D // 2, D), u32))

    cp_wo.wait()
    cp_g.wait()

    def proj_do(sb, c):
        gb = g_buf[pl.ds(pl.multiple_of(sb * TQ, TQ), TQ), D:2 * D]
        dot[:, pl.ds(pl.multiple_of(sb * TQ, TQ), TQ)] = _rnd(_dot(wo_buf[...], gb, NT))
        return c
    lax.fori_loop(0, NQ, proj_do, 0)

    def windows(g, c):
        base = pl.multiple_of(g * 80, 8)
        row = lax.broadcasted_iota(jnp.int32, (R, S), 0)
        zero8 = jnp.zeros((8, S), f32)
        kparts = []
        vparts = []
        for i in range(4):
            a = (0, 16, 40, 56)[i]
            sp = 20 if i % 2 == 0 else 0
            kparts += [qkvt[pl.ds(D + base + a, R), :], zero8]
            vw = qkvt[pl.ds(2 * D + base + a, R), :]
            vw = jnp.where((row >= sp) & (row < sp + 4), 1.0, vw)
            vta[pl.ds(pl.multiple_of((4 * g + i) * R, 8), R), :] = vw
            vparts += [vw, zero8]
        kwin[g] = _pk(jnp.concatenate(kparts, axis=0).astype(bf16).T)
        vwin[g] = _pk(jnp.concatenate(vparts, axis=0).astype(bf16).T)
        return c
    lax.fori_loop(0, NG, windows, 0)

    cp_k.wait()
    cp_v.wait()
    cp_q.wait()
    cp_h.wait()

    def conv_phase(kpad, ksh, kv, dy, dks, uf, gf, hf, skt, red):
        sk = jnp.concatenate([sk_ref[...].astype(f32), jnp.zeros((D, 128 - KS), f32)], axis=1)
        skt[...] = sk.T[0:8, :]
        kpad[0:8, :] = jnp.zeros((8, 128), f32)
        dks[S:S + 8, :] = jnp.zeros((8, 128), f32)
        sgn = jnp.where(lax.broadcasted_iota(jnp.int32, (8, 128), 0) % 2 == 0, 1.0, -1.0)

        def group(cg, c0):
            ln = pl.ds(pl.multiple_of(cg * 128, 128), 128)
            wj = [skt[j:j + 1, ln] for j in range(KS)]
            dvec = ssmd_ref[:, ln].astype(f32)
            kpad[8:8 + S, :] = k_buf[:, ln].astype(f32)

            def fwd(b4, c):
                r0 = pl.multiple_of(b4 * 512, 512)
                kp = kpad[pl.ds(r0, 520), :]
                s = kp[8:520] * wj[0]
                for j in range(1, KS):
                    s = s + kp[8 - j:520 - j] * wj[j]
                rows = pl.ds(r0, 512)
                ksh[rows, :] = s
                u = _rnd(s * v_buf[rows, ln].astype(f32))
                kv[rows, :] = u
                g = _rnd(g_buf[rows, ln].astype(f32) * q_buf[rows, ln].astype(f32))
                dy[rows, :] = g
                fw = fw_ref[...]
                ub = jnp.concatenate([u[i * BL:(i + 1) * BL] for i in range(4)], axis=1).astype(bf16)
                gb = jnp.concatenate([g[i * BL:(i + 1) * BL] for i in range(4)], axis=1).astype(bf16)
                hrow = h_buf[ln, pl.ds(r0, 512)]
                hb = jnp.concatenate([hrow[:, i * BL:(i + 1) * BL] for i in range(4)], axis=0)
                ru = _dot(fw, ub, NN)
                rg = _dot(fw, gb, NN)
                rh = _dot(fw, hb, NT)
                for i in range(4):
                    uf[b4 * 4 + i] = ru[:, i * 128:(i + 1) * 128]
                    gf[b4 * 4 + i] = rg[:, i * 128:(i + 1) * 128]
                    hf[b4 * 4 + i] = rh[:, i * 128:(i + 1) * 128]
                return c
            lax.fori_loop(0, NB // 4, fwd, 0)

            def freq(fg, c):
                re = pl.ds(pl.multiple_of(fg * 8, 8), 8)
                im = pl.ds(pl.multiple_of(BL + fg * 8, 8), 8)
                hr0 = [hf[m, re, :] for m in range(NB)]
                hi0 = [hf[m, im, :] for m in range(NB)]
                hr = [hr0[0]] + [hr0[m] - sgn * hi0[m - 1] for m in range(1, NB)]
                hi = [hi0[0]] + [hi0[m] + sgn * hr0[m - 1] for m in range(1, NB)]
                ur = [uf[m, re, :] for m in range(NB)]
                ui = [uf[m, im, :] for m in range(NB)]
                gr = [gf[m, re, :] for m in range(NB)]
                gi = [gf[m, im, :] for m in range(NB)]
                zr, zi, dr, di, cr, ci = [], [], [], [], [], []
                for i in range(NB):
                    ar = ai = None
                    for m in range(i + 1):
                        tr = hr[m] * ur[i - m] - hi[m] * ui[i - m]
                        ti = hr[m] * ui[i - m] + hi[m] * ur[i - m]
                        ar = tr if ar is None else ar + tr
                        ai = ti if ai is None else ai + ti
                    zr.append(ar)
                    zi.append(ai)
                for j in range(NB):
                    ar = ai = None
                    for m in range(NB - j):
                        tr = hr[m] * gr[j + m] + hi[m] * gi[j + m]
                        ti = hr[m] * gi[j + m] - hi[m] * gr[j + m]
                        ar = tr if ar is None else ar + tr
                        ai = ti if ai is None else ai + ti
                    dr.append(ar)
                    di.append(ai)
                for m in range(NB):
                    ar = ai = None
                    for i in range(m, NB):
                        tr = ur[i - m] * gr[i] + ui[i - m] * gi[i]
                        ti = ur[i - m] * gi[i] - ui[i - m] * gr[i]
                        ar = tr if ar is None else ar + tr
                        ai = ti if ai is None else ai + ti
                    cr.append(ar)
                    ci.append(ai)
                for m in range(NB):
                    uf[m, re, :] = zr[m]
                    uf[m, im, :] = zi[m]
                    gf[m, re, :] = dr[m]
                    gf[m, im, :] = di[m]
                    if m + 1 < NB:
                        hf[m, re, :] = cr[m] + sgn * ci[m + 1]
                        hf[m, im, :] = ci[m] - sgn * cr[m + 1]
                    else:
                        hf[m, re, :] = cr[m]
                        hf[m, im, :] = ci[m]
                return c
            lax.fori_loop(0, BL // 8, freq, 0)

            def inv(b2, acc):
                iv = iv_ref[...]
                zz = jnp.concatenate([uf[2 * b2], uf[2 * b2 + 1], gf[2 * b2], gf[2 * b2 + 1],
                                      hf[2 * b2], hf[2 * b2 + 1]], axis=1).astype(bf16)
                r = _dot(iv, zz, NN)
                r0 = pl.multiple_of(b2 * 256, 256)
                rows = pl.ds(r0, 256)
                yc = jnp.concatenate([r[:, 0:128], r[:, 128:256]], axis=0)
                du = jnp.concatenate([r[:, 256:384], r[:, 384:512]], axis=0)
                dh = jnp.concatenate([r[:, 512:640], r[:, 640:768]], axis=0).astype(bf16)
                h_buf[ln, rows] = dh.T
                u = kv[rows, :]
                g = dy[rows, :]
                y = yc + u * dvec
                qv = q_buf[rows, ln].astype(f32)
                ga = g_buf[rows, ln].astype(f32)
                g_buf[rows, ln] = (qv * y).astype(bf16)
                q_buf[rows, ln] = (ga * y).astype(bf16)
                dkv = g * dvec + du
                dk_s = dkv * v_buf[rows, ln].astype(f32)
                v_buf[rows, ln] = (dkv * ksh[rows, :]).astype(bf16)
                dks[rows, :] = dk_s
                kp = kpad[pl.ds(r0, 264), :]
                new = []
                for j in range(KS):
                    t = dk_s * kp[8 - j:264 - j]
                    new.append(acc[j] + jnp.sum(t.reshape(32, 8, 128), axis=0))
                new.append(acc[KS] + jnp.sum((g * u).reshape(32, 8, 128), axis=0))
                return tuple(new)
            acc = lax.fori_loop(0, NB // 2, inv, tuple(jnp.zeros((8, 128), f32) for _ in range(KS + 1)))
            for j in range(KS + 1):
                red[j:j + 1, ln] = jnp.sum(acc[j], axis=0, keepdims=True)

            def dkpass(b4, c):
                r0 = pl.multiple_of(b4 * 512, 512)
                dp = dks[pl.ds(r0, 520), :]
                s = dp[0:512] * wj[0]
                for j in range(1, KS):
                    s = s + dp[j:512 + j] * wj[j]
                k_buf[pl.ds(r0, 512), ln] = s.astype(bf16)
                return c
            lax.fori_loop(0, NB // 4, dkpass, 0)
            return c0

        red[...] = jnp.zeros((128, D), f32)
        lax.fori_loop(0, NCG, group, 0)
        dssmd_ref[...] = red[KS:KS + 1, :].astype(bf16)
        dsk_ref[...] = red[...].T[:, 0:KS].astype(bf16)

    pl.run_scoped(
        conv_phase,
        pltpu.VMEM((S + 8, 128), f32), pltpu.VMEM((S, 128), f32), pltpu.VMEM((S, 128), f32),
        pltpu.VMEM((S, 128), f32), pltpu.VMEM((S + 8, 128), f32),
        pltpu.VMEM((NB, 2 * BL, 128), f32), pltpu.VMEM((NB, 2 * BL, 128), f32),
        pltpu.VMEM((NB, 2 * BL, 128), f32),
        pltpu.VMEM((8, D), f32), pltpu.VMEM((128, D), f32))

    out_a = [
        pltpu.make_async_copy(q_buf, dq_hbm, sems.at[8]),
        pltpu.make_async_copy(k_buf, dk_hbm, sems.at[9]),
        pltpu.make_async_copy(v_buf, dv_hbm, sems.at[10]),
        pltpu.make_async_copy(h_buf, dssmk_hbm, sems.at[11]),
        pltpu.make_async_copy(g_buf.at[:, 0:D], out_hbm.at[:, 0:D], sems.at[12]),
    ]
    for c in out_a:
        c.start()

    def attn_phase(ot, dqkvt, s_buf, p_buf, wq_buf, wdo_buf, dop_buf, qm_buf, m_buf,
                   acco_buf, accq_buf, mx_buf, ds_buf):
        ot[...] = jnp.zeros_like(ot)
        dqkvt[...] = jnp.zeros_like(dqkvt)
        rowr = lax.broadcasted_iota(jnp.int32, (R, TQ), 0)

        def unit(u):
            h = u // NQ
            a = pl.multiple_of(8 * ((5 * h) // 2), 8)
            q0 = pl.multiple_of((u % NQ) * TQ, TQ)
            off = 4 * (h % 2)
            return h, a, q0, off

        def head_mask(off):
            return (rowr >= off) & (rowr < off + DH)

        def put_block(buf, par, h, blk):
            pb = _pk(jnp.concatenate([blk, jnp.zeros((8, TQ), f32)], axis=0).astype(bf16))
            for i in range(4):
                buf[par, i * 16:(i + 1) * 16, :] = jnp.where(h % 4 == i, pb, jnp.zeros_like(pb))

        def masked_q(u):
            h, a, q0, off = unit(u)
            return jnp.where(head_mask(off), qkvt[pl.ds(a, R), pl.ds(q0, TQ)], 0.0)

        def emit(s_lo, s_hi, ubase, lo_valid, hi_valid):
            st = {}

            def ok(g):
                return lo_valid <= g < hi_valid

            def get(name, buf):
                if name not in st:
                    st[name] = buf[...]
                return st[name]

            for s in range(s_lo, s_hi):
                ds_new = None
                if ok(s):
                    ur, c = divmod(s, NC)
                    par = ur % 2
                    h, a, q0, off = unit(ubase + ur)
                    kh = slice(c * CK // 2, (c + 1) * CK // 2)
                    dp = _dot(_up(vwin[h // 4, kh, :]), _up(wdo_buf[par]), NN)
                    pc = _up(p_buf[par, kh, :])
                    ds_new = (pc.astype(f32) * dp).astype(bf16)
                if ok(s - 1):
                    ur, c = divmod(s - 1, NC)
                    h, a, q0, off = unit(ubase + ur)
                    ks = slice(c * CK, (c + 1) * CK)
                    if c == 0:
                        qm_buf[...] = masked_q(ubase + ur)
                    dsp = st['ds'] if 'ds' in st else _up(ds_buf[...])
                    dqkvt[pl.ds(D + a, R), ks] += _dot(qm_buf[...], dsp, NT)
                    t = _dot(qkvt[pl.ds(D + a, R), ks], dsp, NN)
                    st['accq'] = t if c == 0 else get('accq', accq_buf) + t
                    if c == NC - 1:
                        dqkvt[pl.ds(a, R), pl.ds(q0, TQ)] += jnp.where(head_mask(off), st['accq'] * SCALE, 0.0)
                if ds_new is not None:
                    st['ds'] = ds_new
                if ok(s + OFF_A):
                    ur, c = divmod(s + OFF_A, NC)
                    par = ur % 2
                    h, a, q0, off = unit(ubase + ur)
                    if c == 0:
                        put_block(wq_buf, par, h, masked_q(ubase + ur))
                    kh = slice(c * CK // 2, (c + 1) * CK // 2)
                    sc = _dot(_up(kwin[h // 4, kh, :]), _up(wq_buf[par]), NN)
                    s_buf[par, c * CK:(c + 1) * CK, :] = sc
                    t = jnp.max(sc.reshape(CK // 8, 8, TQ), axis=0)
                    st['mx'] = t if c == 0 else jnp.maximum(get('mx', mx_buf), t)
                    if c == NC - 1:
                        m_buf[par] = jnp.broadcast_to(jnp.max(st['mx'], axis=0, keepdims=True), (8, TQ))
                if ok(s):
                    ur, c = divmod(s, NC)
                    par = ur % 2
                    h, a, q0, off = unit(ubase + ur)
                    dqkvt[pl.ds(2 * D + a, R), c * CK:(c + 1) * CK] += _dot(dop_buf[par], pc, NT)
                if ok(s + OFF_E):
                    ur, c = divmod(s + OFF_E, NC)
                    par = ur % 2
                    sc = s_buf[par, c * CK:(c + 1) * CK, :].reshape(CK // 8, 8, TQ)
                    p = jnp.exp2(sc - m_buf[par][None]).reshape(CK, TQ)
                    p_buf[par, c * CK // 2:(c + 1) * CK // 2, :] = _pk(p.astype(bf16))
                if ok(s + OFF_O):
                    ur, c = divmod(s + OFF_O, NC)
                    par = ur % 2
                    h, a, q0, off = unit(ubase + ur)
                    va = vta[pl.ds(pl.multiple_of(h * R, 8), R), c * CK:(c + 1) * CK]
                    t = _dot(va, _up(p_buf[par, c * CK // 2:(c + 1) * CK // 2, :]), NN)
                    st['acco'] = t if c == 0 else get('acco', acco_buf) + t
                    if c == NC - 1:
                        acco = st['acco']
                        sp = 20 - 5 * off
                        hm = head_mask(off)
                        l = jnp.sum(jnp.where(rowr == sp, acco, 0.0), axis=0, keepdims=True)
                        inv = 1.0 / l
                        o = jnp.where(hm, acco * inv, 0.0)
                        ot[pl.ds(a, R), pl.ds(q0, TQ)] += o
                        do = jnp.where(hm, dot[pl.ds(a, R), pl.ds(q0, TQ)], 0.0)
                        delta = jnp.sum(do * o, axis=0, keepdims=True) * inv
                        dop = _rnd(do * inv)
                        dop_buf[par] = dop
                        dhi = _rnd(delta)
                        blk = jnp.where(rowr == sp, -dhi, jnp.where(rowr == sp + 1, dhi - delta, dop))
                        put_block(wdo_buf, par, h, blk)
            if 'ds' in st:
                ds_buf[...] = _pk(st['ds'])
            if 'accq' in st:
                accq_buf[...] = st['accq']
            if 'acco' in st:
                acco_buf[...] = st['acco']
            if 'mx' in st:
                mx_buf[...] = st['mx']

        big = 1 << 30
        emit(-OFF_A, S0, 0, 0, big)

        def body(it, c):
            emit(S0, S0 + UNR * NC, UNR * it, -big, big)
            return c
        lax.fori_loop(0, NIT, body, 0)
        ub = UNR * NIT
        emit(S0, (NU - ub) * NC + 1, ub, -big, (NU - ub) * NC)

        def out_phase(xt, dg, ob):
            def cast(j, c):
                rows = pl.ds(pl.multiple_of(j * 128, 128), 128)
                sc = jnp.where(j // NCG == 1, 1.0 / LOG2E, 1.0)
                dg[pl.ds(pl.multiple_of(j * 64, 64), 64), :] = _pk((dqkvt[rows, :] * sc).astype(bf16))
                return c
            lax.fori_loop(0, 3 * NCG, cast, 0)

            def casto(j, c):
                rows = pl.ds(pl.multiple_of(j * 128, 128), 128)
                ob[pl.ds(pl.multiple_of(j * 64, 64), 64), :] = _pk(ot[rows, :].astype(bf16))
                xt[pl.ds(pl.multiple_of(j * 64, 64), 64), :] = _pk(x_buf[:, rows].T)
                return c
            lax.fori_loop(0, NCG, casto, 0)

            dwo = _dot(_up(ob[...]), g_buf[:, D:2 * D], NN)
            ot[:, 0:D] = dwo

            def outb(sb, c):
                cols = pl.ds(pl.multiple_of(sb * TQ, TQ), TQ)
                o = _up(ob[:, cols]).T
                g_buf[cols, D:2 * D] = _dot(o, wo_buf[...], NN).astype(bf16)
                dxt = _dot(w_buf[...], _up(dg[:, cols]), NN)
                x_buf[cols, :] = dxt.astype(bf16).T
                return c
            lax.fori_loop(0, NQ, outb, 0)
            wo_buf[...] = ot[:, 0:D].astype(bf16)
            cps = [
                pltpu.make_async_copy(g_buf.at[:, D:2 * D], out_hbm.at[:, D:2 * D], sems.at[13]),
                pltpu.make_async_copy(x_buf, dx_hbm, sems.at[14]),
                pltpu.make_async_copy(wo_buf, dwo_hbm, sems.at[15]),
            ]
            for c in cps:
                c.start()

            def dw(j, c):
                rows = pl.ds(pl.multiple_of(j * 192, 64), 192)
                r = _dot(_up(xt[...]), _up(dg[rows, :]), NT)
                w_buf[:, pl.ds(pl.multiple_of(j * 384, 128), 384)] = r.astype(bf16)
                return c
            lax.fori_loop(0, 5, dw, 0)
            cpw = pltpu.make_async_copy(w_buf, dwqkv_hbm, sems.at[16])
            cpw.start()
            for c in cps:
                c.wait()
            cpw.wait()

        pl.run_scoped(out_phase, pltpu.VMEM((D // 2, S), u32), pltpu.VMEM((3 * D // 2, S), u32),
                      pltpu.VMEM((D // 2, S), u32))

    pl.run_scoped(
        attn_phase,
        pltpu.VMEM((D, S), f32), pltpu.VMEM((3 * D, S), f32),
        pltpu.VMEM((2, S, TQ), f32), pltpu.VMEM((2, S // 2, TQ), u32),
        pltpu.VMEM((2, 64, TQ), u32), pltpu.VMEM((2, 64, TQ), u32),
        pltpu.VMEM((2, R, TQ), f32), pltpu.VMEM((R, TQ), f32), pltpu.VMEM((2, 8, TQ), f32),
        pltpu.VMEM((R, TQ), f32), pltpu.VMEM((R, TQ), f32), pltpu.VMEM((8, TQ), f32),
        pltpu.VMEM((CK // 2, TQ), u32))

    for c in out_a:
        c.wait()


@jax.jit
def pallas_concat_heads__ssm_conv_h3__softmax_full_mha__prompt_kernel(
    A_q: jax.Array,
    A_k: jax.Array,
    A_v: jax.Array,
    A_shift_k: jax.Array,
    A_ssm_k: jax.Array,
    A_ssm_D: jax.Array,
    B_x: jax.Array,
    B_wqkv: jax.Array,
    B_wo: jax.Array,
    grad_out: jax.Array,
):
    fw, iv = _dft_mats()
    fw = jnp.asarray(fw, dtype=bf16)
    iv = jnp.asarray(iv, dtype=bf16)
    hbm = pl.BlockSpec(memory_space=pl.ANY)
    vmem = pl.BlockSpec(memory_space=pltpu.VMEM)
    sd = jax.ShapeDtypeStruct
    outs = pl.pallas_call(
        _kernel,
        in_specs=[hbm, hbm, hbm, vmem, hbm, vmem, hbm, hbm, hbm, hbm, vmem, vmem],
        out_specs=[hbm, hbm, hbm, hbm, vmem, hbm, vmem, hbm, hbm, hbm],
        out_shape=[sd((S, 2 * D), bf16), sd((S, D), bf16), sd((S, D), bf16), sd((S, D), bf16),
                   sd((D, KS), bf16), sd((D, S), bf16), sd((1, D), bf16), sd((S, D), bf16),
                   sd((D, 3 * D), bf16), sd((D, D), bf16)],
        scratch_shapes=[
            pltpu.VMEM((S, D), bf16), pltpu.VMEM((S, D), bf16), pltpu.VMEM((S, D), bf16),
            pltpu.VMEM((D, S), bf16), pltpu.VMEM((S, D), bf16), pltpu.VMEM((D, 3 * D), bf16),
            pltpu.VMEM((D, D), bf16), pltpu.VMEM((S, 2 * D), bf16),
            pltpu.VMEM((3 * D, S), f32), pltpu.VMEM((D, S), f32), pltpu.VMEM((H * R, S), f32),
            pltpu.VMEM((NG, S // 2, 128), u32), pltpu.VMEM((NG, S // 2, 128), u32),
            pltpu.SemaphoreType.DMA((17,)),
        ],
        compiler_params=pltpu.CompilerParams(vmem_limit_bytes=120 * 1024 * 1024),
    )(A_q.reshape(S, D), A_k.reshape(S, D), A_v.reshape(S, D), A_shift_k, A_ssm_k,
      A_ssm_D.reshape(1, D), B_x.reshape(S, D), B_wqkv, B_wo, grad_out.reshape(S, 2 * D), fw, iv)
    out, dq, dk, dv, dsk, dssmk, dssmd, dx, dwqkv, dwo = outs
    return (out.reshape(1, S, 2 * D), dq.reshape(1, S, D), dk.reshape(1, S, D), dv.reshape(1, S, D),
            dsk, dssmk, dssmd.reshape(D), dx.reshape(1, S, D), dwqkv, dwo)
```

```python
import math

import numpy as np
import jax
import jax.numpy as jnp
from jax import lax
import jax.experimental.pallas as pl
import jax.experimental.pallas.tpu as pltpu

S = 2048
D = 640
H = 32
DH = 20
KS = 4
TQ = 512
CK = 128
R = 24
HP = H * R
NQ = S // TQ
NC = S // CK
NU = H * NQ
BL = 128
NB = S // BL
W1 = 256
W2 = D - W1

OFF_O = 18
S0 = 5
VL = 1
NVG = 32
NVC = NVG // 8
VPASS = [range(j * 2 * NVG // NC, (j + 1) * 2 * NVG // NC) for j in range(NC)]
MGRP = [range(NVG + j * (S // 16 - NVG) // NC, NVG + (j + 1) * (S // 16 - NVG) // NC) for j in range(NC)]
_GDONE = {p // 2: j for j in range(NC) for p in VPASS[j]}
_GDONE.update({g: j for j in range(NC) for g in MGRP[j]})
_DONE = [max(_GDONE[g] for g in range(8 * c, 8 * c + 8)) for c in range(NC)]
ORDER = sorted(range(NC), key=lambda c: (_DONE[c], -c))
LEAD = max(_DONE[c] - n for n, c in enumerate(ORDER)) + 1
OFF_A = OFF_O + LEAD
NIT = (NU * NC - OFF_A - VL - S0) // (NQ * NC)
NTS = 22
NCE = H - 4
NCS = 21
SAFE = 20.0

f32 = jnp.float32
bf16 = jnp.bfloat16
u32 = jnp.uint32
NN = (((1,), (0,)), ((), ()))
NT = (((1,), (1,)), ((), ()))

SCALE = float(DH) ** -0.5
QS = SCALE * math.log2(math.e)


def _dot(a, b, dims):
    return lax.dot_general(a, b, dims, preferred_element_type=f32)


def _up(x):
    return pltpu.bitcast(x, bf16)


def _pk(x):
    return pltpu.bitcast(x, u32)


def _ds(start, size, mult):
    return pl.ds(pl.multiple_of(start, mult), size)


def _tile(x, rows, cols):
    if cols > 1:
        x = jnp.concatenate([x] * cols, axis=1)
    if rows > 1:
        x = jnp.concatenate([x] * rows, axis=0)
    return x


def _dft_mats():
    f = np.arange(BL, dtype=np.float64)[:, None] + 0.5
    n = np.arange(BL, dtype=np.float64)[None, :]
    th = 2.0 * np.pi * f * n / (2 * BL)
    fwd = np.concatenate([np.cos(th), -np.sin(th)], axis=0)
    inv = fwd.T / BL
    perm = np.concatenate([np.concatenate([np.arange(8 * j, 8 * j + 8), BL + np.arange(8 * j, 8 * j + 8)])
                           for j in range(BL // 8)])
    return fwd[perm].astype(np.float32), inv[:, perm].astype(np.float32)


class _Pins:
    def __init__(self, items=()):
        self.items = list(items)

    def add(self, t, lanes=1):
        self.items += [(t, k, n) for n in range(lanes) for k in range(t.shape[0] // 8)]

    def window(self, lo, hi):
        return _Pins([None] * max(0, -lo) + self.items[max(lo, 0):hi])

    def at(self, num, den):
        if not self.items:
            return None
        it = self.items[min(len(self.items) - 1, len(self.items) * num // den)]
        if it is None:
            return None
        t, k, n = it
        return t[8 * k:8 * k + 8, 128 * n:128 * n + 128]


def _roomy(fn, *args):
    if fn is None:
        (_, _, _, _, _, _, _, _, _, _, _, _, _, _, _, _, _, _, _, _, _, _, _, _, _, _, _, _, _, _, _, _,
         _, _, _, _, _, _, _, _, _, _, _, _, _, _, _, _, _, _, _, _, _, _, _, _, _, _, _, _, _, _, _, _,
         _, _, _, _, _, _, _, _, _, _, _, _, _, _, _, _, _, _, _, _, _, _, _, _, _, _, _, _, _, _, _, _,
         _, _, _, _, _, _, _, _, _, _, _, _, _, _, _, _, _, _, _, _, _, _, _, _, _, _, _, _, _, _, _, _,
         _, _, _, _, _, _, _, _, _, _, _, _, _, _, _, _, _, _, _, _, _, _, _, _, _, _, _, _, _, _, _, _,
         _, _, _, _, _, _, _, _, _, _, _, _, _, _, _, _, _, _, _, _, _, _, _, _, _, _, _, _, _, _, _, _,
         _, _, _, _, _, _, _, _, _, _, _, _, _, _, _, _, _, _, _, _, _, _, _, _, _, _, _, _, _, _, _, _,
         _, _, _, _, _, _, _, _, _, _, _, _, _, _, _, _, _, _, _, _, _, _, _, _, _, _, _, _, _, _, _, _,
         _, _, _, _, _, _, _, _, _, _, _, _, _, _, _, _, _, _, _, _, _, _, _, _, _, _, _, _, _, _, _, _,
         _, _, _, _, _, _, _, _, _, _, _, _, _, _, _, _, _, _, _, _, _, _, _, _, _, _, _, _, _, _, _, _,
         _, _, _, _, _, _, _, _, _, _, _, _, _, _, _, _, _, _, _, _, _, _, _, _, _, _, _, _, _, _, _, _,
         _, _, _, _, _, _, _, _, _, _, _, _, _, _, _, _, _, _, _, _, _, _, _, _, _, _, _, _, _, _, _, _,
         _, _, _, _, _, _, _, _, _, _, _, _, _, _, _, _, _, _, _, _, _, _, _, _, _, _, _, _, _, _, _, _,
         _, _, _, _, _, _, _, _, _, _, _, _, _, _, _, _, _, _, _, _, _, _, _, _, _, _, _, _, _, _, _, _,
         _, _, _, _, _, _, _, _, _, _, _, _, _, _, _, _, _, _, _, _, _, _, _, _, _, _, _, _, _, _, _, _,
         _, _, _, _, _, _, _, _, _, _, _, _, _, _, _, _, _, _, _, _, _, _, _, _, _, _, _, _, _, _, _, _,
         _, _, _, _, _, _, _, _, _, _, _, _, _, _, _, _, _, _, _, _, _, _, _, _, _, _, _, _, _, _, _, _,
         _, _, _, _, _, _, _, _, _, _, _, _, _, _, _, _, _, _, _, _, _, _, _, _, _, _, _, _, _, _, _, _,
         _, _, _, _, _, _, _, _, _, _, _, _, _, _, _, _, _, _, _, _, _, _, _, _, _, _, _, _, _, _, _, _,
         _, _, _, _, _, _, _, _, _, _, _, _, _, _, _, _, _, _, _, _, _, _, _, _, _, _, _, _, _, _, _, _,
         _, _, _, _, _, _, _, _, _, _, _, _, _, _, _, _, _, _, _, _, _, _, _, _, _, _, _, _, _, _, _, _,
         _, _, _, _, _, _, _, _, _, _, _, _, _, _, _, _, _, _, _, _, _, _, _, _, _, _, _, _, _, _, _, _,
         _, _, _, _, _, _, _, _, _, _, _, _, _, _, _, _, _, _, _, _, _, _, _, _, _, _, _, _, _, _, _, _,
         _, _, _, _, _, _, _, _, _, _, _, _, _, _, _, _, _, _, _, _, _, _, _, _, _, _, _, _, _, _, _, _,
         _, _, _, _, _, _, _, _, _, _, _, _, _, _, _, _, _, _, _, _, _, _, _, _, _, _, _, _, _, _, _, _,
         _, _, _, _, _, _, _, _, _, _, _, _, _, _, _, _, _, _, _, _, _, _, _, _, _, _, _, _, _, _, _, _,
         _, _, _, _, _, _, _, _, _, _, _, _, _, _, _, _, _, _, _, _, _, _, _, _, _, _, _, _, _, _, _, _,
         _, _, _, _, _, _, _, _, _, _, _, _, _, _, _, _, _, _, _, _, _, _, _, _, _, _, _, _, _, _, _, _,
         _, _, _, _, _, _, _, _, _, _, _, _, _, _, _, _, _, _, _, _, _, _, _, _, _, _, _, _, _, _, _, _,
         _, _, _, _, _, _, _, _, _, _, _, _, _, _, _, _, _, _, _, _, _, _, _, _, _, _, _, _, _, _, _, _,
         _, _, _, _, _, _, _, _, _, _, _, _, _, _, _, _, _, _, _, _, _, _, _, _, _, _, _, _, _, _, _, _,
         _, _, _, _, _, _, _, _, _, _, _, _, _, _, _, _, _, _, _, _, _, _, _, _, _, _, _, _, _, _, _, _,
         _, _, _, _, _, _, _, _, _, _, _, _, _, _, _, _, _, _, _, _, _, _, _, _, _, _, _, _, _, _, _, _,
         _, _, _, _, _, _, _, _, _, _, _, _, _, _, _, _, _, _, _, _, _, _, _, _, _, _, _, _, _, _, _, _,
         _, _, _, _, _, _, _, _, _, _, _, _, _, _, _, _, _, _, _, _, _, _, _, _, _, _, _, _, _, _, _, _,
         _, _, _, _, _, _, _, _, _, _, _, _, _, _, _, _, _, _, _, _, _, _, _, _, _, _, _, _, _, _, _, _,
         _, _, _, _, _, _, _, _, _, _, _, _, _, _, _, _, _, _, _, _, _, _, _, _, _, _, _, _, _, _, _, _,
         _, _, _, _, _, _, _, _, _, _, _, _, _, _, _, _, _, _, _, _, _, _, _, _, _, _, _, _, _, _, _, _,
         _, _, _, _, _, _, _, _, _, _, _, _, _, _, _, _, _, _, _, _, _, _, _, _, _, _, _, _, _, _, _, _,
         _, _, _, _, _, _, _, _, _, _, _, _, _, _, _, _, _, _, _, _, _, _, _, _, _, _, _, _, _, _, _, _,
         _, _, _, _, _, _, _, _, _, _, _, _, _, _, _, _, _, _, _, _, _, _, _, _, _, _, _, _, _, _, _, _,
         _, _, _, _, _, _, _, _, _, _, _, _, _, _, _, _, _, _, _, _, _, _, _, _, _, _, _, _, _, _, _, _,
         _, _, _, _, _, _, _, _, _, _, _, _, _, _, _, _, _, _, _, _, _, _, _, _, _, _, _, _, _, _, _, _,
         _, _, _, _, _, _, _, _, _, _, _, _, _, _, _, _, _, _, _, _, _, _, _, _, _, _, _, _, _, _, _, _,
         _, _, _, _, _, _, _, _, _, _, _, _, _, _, _, _, _, _, _, _, _, _, _, _, _, _, _, _, _, _, _, _,
         _, _, _, _, _, _, _, _, _, _, _, _, _, _, _, _, _, _, _, _, _, _, _, _, _, _, _, _, _, _, _, _,
         _, _, _, _, _, _, _, _, _, _, _, _, _, _, _, _, _, _, _, _, _, _, _, _, _, _, _, _, _, _, _, _,
         _, _, _, _, _, _, _, _, _, _, _, _, _, _, _, _, _, _, _, _, _, _, _, _, _, _, _, _, _, _, _, _,
         _, _, _, _, _, _, _, _, _, _, _, _, _, _, _, _, _, _, _, _, _, _, _, _, _, _, _, _, _, _, _, _,
         _, _, _, _, _, _, _, _, _, _, _, _, _, _, _, _, _, _, _, _, _, _, _, _, _, _, _, _, _, _, _, _,
         _, _, _, _, _, _, _, _, _, _, _, _, _, _, _, _, _, _, _, _, _, _, _, _, _, _, _, _, _, _, _, _,
         _, _, _, _, _, _, _, _, _, _, _, _, _, _, _, _, _, _, _, _, _, _, _, _, _, _, _, _, _, _, _, _,
         _, _, _, _, _, _, _, _, _, _, _, _, _, _, _, _, _, _, _, _, _, _, _, _, _, _, _, _, _, _, _, _,
         _, _, _, _, _, _, _, _, _, _, _, _, _, _, _, _, _, _, _, _, _, _, _, _, _, _, _, _, _, _, _, _,
         _, _, _, _, _, _, _, _, _, _, _, _, _, _, _, _, _, _, _, _, _, _, _, _, _, _, _, _, _, _, _, _,
         _, _, _, _, _, _, _, _, _, _, _, _, _, _, _, _, _, _, _, _, _, _, _, _, _, _, _, _, _, _, _, _,
         _, _, _, _, _, _, _, _, _, _, _, _, _, _, _, _, _, _, _, _, _, _, _, _, _, _, _, _, _, _, _, _,
         _, _, _, _, _, _, _, _, _, _, _, _, _, _, _, _, _, _, _, _, _, _, _, _, _, _, _, _, _, _, _, _,
         _, _, _, _, _, _, _, _, _, _, _, _, _, _, _, _, _, _, _, _, _, _, _, _, _, _, _, _, _, _, _, _,
         _, _, _, _, _, _, _, _, _, _, _, _, _, _, _, _, _, _, _, _, _, _, _, _, _, _, _, _, _, _, _, _,
         _, _, _, _, _, _, _, _, _, _, _, _, _, _, _, _, _, _, _, _, _, _, _, _, _, _, _, _, _, _, _, _,
         _, _, _, _, _, _, _, _, _, _, _, _, _, _, _, _, _, _, _, _, _, _, _, _, _, _, _, _, _, _, _, _,
         _, _, _, _, _, _, _, _, _, _, _, _, _, _, _, _, _, _, _, _, _, _, _, _, _, _, _, _, _, _, _, _,
         _, _, _, _, _, _, _, _, _, _, _, _, _, _, _, _, _, _, _, _, _, _, _, _, _, _, _, _, _, _, _, _,
         _, _, _, _, _, _, _, _, _, _, _, _, _, _, _, _, _, _, _, _, _, _, _, _, _, _, _, _, _, _, _, _,
         _, _, _, _, _, _, _, _, _, _, _, _, _, _, _, _, _, _, _, _, _, _, _, _, _, _, _, _, _, _, _, _,
         _, _, _, _, _, _, _, _, _, _, _, _, _, _, _, _, _, _, _, _, _, _, _, _, _, _, _, _, _, _, _, _,
         _, _, _, _, _, _, _, _, _, _, _, _, _, _, _, _, _, _, _, _, _, _, _, _, _, _, _, _, _, _, _, _,
         _, _, _, _, _, _, _, _, _, _, _, _, _, _, _, _, _, _, _, _, _, _, _, _, _, _, _, _, _, _, _, _,
         _, _, _, _, _, _, _, _, _, _, _, _, _, _, _, _, _, _, _, _, _, _, _, _, _, _, _, _, _, _, _, _,
         _, _, _, _, _, _, _, _, _, _, _, _, _, _, _, _, _, _, _, _, _, _, _, _, _, _, _, _, _, _, _, _,
         _, _, _, _, _, _, _, _, _, _, _, _, _, _, _, _, _, _, _, _, _, _, _, _, _, _, _, _, _, _, _, _,
         _, _, _, _, _, _, _, _, _, _, _, _, _, _, _, _, _, _, _, _, _, _, _, _, _, _, _, _, _, _, _, _,
         _, _, _, _, _, _, _, _, _, _, _, _, _, _, _, _, _, _, _, _, _, _, _, _, _, _, _, _, _, _, _, _,
         _, _, _, _, _, _, _, _, _, _, _, _, _, _, _, _, _, _, _, _, _, _, _, _, _, _, _, _, _, _, _, _,
         _, _, _, _, _, _, _, _, _, _, _, _, _, _, _, _, _, _, _, _, _, _, _, _, _, _, _, _, _, _, _, _,
         _, _, _, _, _, _, _, _, _, _, _, _, _, _, _, _, _, _, _, _, _, _, _, _, _, _, _, _, _, _, _, _,
         _, _, _, _, _, _, _, _, _, _, _, _, _, _, _, _, _, _, _, _, _, _, _, _, _, _, _, _, _, _, _, _,
         _, _, _, _, _, _, _, _, _, _, _, _, _, _, _, _, _, _, _, _, _, _, _, _, _, _, _, _, _, _, _, _,
         _, _, _, _, _, _, _, _, _, _, _, _, _, _, _, _, _, _, _, _, _, _, _, _, _, _, _, _, _, _, _, _,
         _, _, _, _, _, _, _, _, _, _, _, _, _, _, _, _, _, _, _, _, _, _, _, _, _, _, _, _, _, _, _, _,
         _, _, _, _, _, _, _, _, _, _, _, _, _, _, _, _, _, _, _, _, _, _, _, _, _, _, _, _, _, _, _, _,
         _, _, _, _, _, _, _, _, _, _, _, _, _, _, _, _, _, _, _, _, _, _, _, _, _, _, _, _, _, _, _, _,
         _, _, _, _, _, _, _, _, _, _, _, _, _, _, _, _, _, _, _, _, _, _, _, _, _, _, _, _, _, _, _, _,
         _, _, _, _, _, _, _, _, _, _, _, _, _, _, _, _, _, _, _, _, _, _, _, _, _, _, _, _, _, _, _, _,
         _, _, _, _, _, _, _, _, _, _, _, _, _, _, _, _, _, _, _, _, _, _, _, _, _, _, _, _, _, _, _, _,
         _, _, _, _, _, _, _, _, _, _, _, _, _, _, _, _, _, _, _, _, _, _, _, _, _, _, _, _, _, _, _, _,
         _, _, _, _, _, _, _, _, _, _, _, _, _, _, _, _, _, _, _, _, _, _, _, _, _, _, _, _, _, _, _, _,
         _, _, _, _, _, _, _, _, _, _, _, _, _, _, _, _, _, _, _, _, _, _, _, _, _, _, _, _, _, _, _, _,
         _, _, _, _, _, _, _, _, _, _, _, _, _, _, _, _, _, _, _, _, _, _, _, _, _, _, _, _, _, _, _, _,
         _, _, _, _, _, _, _, _, _, _, _, _, _, _, _, _, _, _, _, _, _, _, _, _, _, _, _, _, _, _, _, _,
         _, _, _, _, _, _, _, _, _, _, _, _, _, _, _, _, _, _, _, _, _, _, _, _, _, _, _, _, _, _, _, _,
         _, _, _, _, _, _, _, _, _, _, _, _, _, _, _, _, _, _, _, _, _, _, _, _, _, _, _, _, _, _, _, _,
         _, _, _, _, _, _, _, _, _, _, _, _, _, _, _, _, _, _, _, _, _, _, _, _, _, _, _, _, _, _, _, _,
         _, _, _, _, _, _, _, _, _, _, _, _, _, _, _, _, _, _, _, _, _, _, _, _, _, _, _, _, _, _, _, _,
         _, _, _, _, _, _, _, _, _, _, _, _, _, _, _, _, _, _, _, _, _, _, _, _, _, _, _, _, _, _, _, _,
         _, _, _, _, _, _, _, _, _, _, _, _, _, _, _, _, _, _, _, _, _, _, _, _, _, _, _, _, _, _, _, _,
         _, _, _, _, _, _, _, _, _, _, _, _, _, _, _, _, _, _, _, _, _, _, _, _, _, _, _, _, _, _, _, _,) = args
    return fn(*args)


def _kernel(*refs):
    _roomy(_body, *refs)


def _body(z_ref, q_hbm, k_hbm, v_hbm, sk_hbm, ssmk_hbm, ssmd_hbm, x_hbm, wqkv_hbm, wo_hbm, g_hbm,
            fw_hbm, iv_hbm,
            out_hbm, dq_hbm, dk_hbm, dv_hbm, dsk_hbm, dssmk_hbm, dssmd_hbm, dx_hbm, dwqkv_hbm,
            dwo_hbm,
            skt, q_buf, k_buf, v_buf, ga_buf, h_buf, xg_buf, w_buf, wo_buf, dwo_buf,
            res, xt, dg, red, amax, fw_ref, iv_ref, drow, sk_ref, ssmd_ref, flag, sems):
    never = z_ref[0] != 0

    def pinned(x, pin):
        if pin is None:
            return x
        return lax.select_n(never, x, _tile(pin, x.shape[0] // pin.shape[0], x.shape[1] // 128))

    SEM_SM, SEM_W, SEM_C1, SEM_X, SEM_MID, SEM_C2, SEM_OUT = 0, 1, 2, 6, 10, 11, 12

    def cp(src, dst, sem):
        return pltpu.make_async_copy(src, dst, sems.at[sem])

    def conv_in(c0, w, r0, n, sem):
        rows = pl.ds(r0, n)
        cols = slice(c0, c0 + w)
        return [cp(k_hbm.at[rows, cols], k_buf.at[rows, cols], sem),
                cp(v_hbm.at[rows, cols], v_buf.at[rows, cols], sem),
                cp(q_hbm.at[rows, cols], q_buf.at[rows, cols], sem),
                cp(g_hbm.at[rows, cols], ga_buf.at[rows, cols], sem),
                cp(ssmk_hbm.at[cols, rows], h_buf.at[cols, rows], sem)]

    def conv_out(c0, w, r0, n):
        rows = pl.ds(r0, n)
        cols = slice(c0, c0 + w)
        return [cp(k_buf.at[rows, cols], dk_hbm.at[rows, cols], SEM_OUT),
                cp(v_buf.at[rows, cols], dv_hbm.at[rows, cols], SEM_OUT),
                cp(q_buf.at[rows, cols], dq_hbm.at[rows, cols], SEM_OUT),
                cp(ga_buf.at[rows, cols], out_hbm.at[rows, cols], SEM_OUT),
                cp(h_buf.at[cols, rows], dssmk_hbm.at[cols, rows], SEM_OUT)]

    def x_in(i):
        rows = _ds(i * TQ, TQ, TQ)
        return cp(x_hbm.at[rows, :], xg_buf.at[rows, :], SEM_X + i)

    cp_small = [cp(sk_hbm, sk_ref, SEM_SM), cp(fw_hbm, fw_ref, SEM_SM),
                cp(ssmd_hbm, ssmd_ref, SEM_SM), cp(iv_hbm, iv_ref, SEM_SM)]
    cp_w = cp(wqkv_hbm.at[:, 0:2 * D], w_buf.at[:, 0:2 * D], SEM_W)
    cp_mid = [cp(wqkv_hbm.at[:, 2 * D:3 * D], w_buf.at[:, 2 * D:3 * D], SEM_MID),
              cp(wo_hbm, wo_buf, SEM_MID),
              cp(g_hbm.at[:, D:2 * D], xg_buf.at[S:2 * S, :], SEM_MID)]
    cp_c2 = conv_in(W1, W2, 0, S, SEM_C2)
    for c in ([cp_w] + cp_small + [c for b in range(4) for c in conv_in(0, W1, b * 512, 512, SEM_C1 + b)]
              + [x_in(i) for i in range(NQ)] + cp_mid + cp_c2):
        c.start()

    def conv_fwd(c0, w, uf, gf, hf, ksh, tb, wait):
        cols = slice(c0, c0 + w)
        wj = [skt[j:j + 1, cols] for j in range(KS)]
        n = tb * BL

        def body(b, kprev):
            r0 = pl.multiple_of(b * n, n)
            if wait:
                for c in conv_in(c0, w, r0, n, SEM_C1 + b):
                    c.wait()
            fw = fw_ref[...]
            for i in range(tb):
                rows = _ds(r0 + i * BL, BL, BL)
                dst = _ds((b * tb + i) * 16, (BL // 8 - 1) * NB * 16 + 16, 16)

                def scatter(ref, val):
                    v = ref.at[dst, :]
                    for fg in range(BL // 8):
                        v[fg * NB * 16:fg * NB * 16 + 16, :] = val[fg * 16:(fg + 1) * 16]
                scatter(hf, _dot(fw, h_buf[cols, rows], NT))
                kf = k_buf[rows, cols].astype(f32)
                kp = jnp.concatenate([kprev, kf], axis=0)
                s = kf * wj[0]
                for j in range(1, KS):
                    s = s + pltpu.roll(kp, j, 0)[8:] * wj[j]
                ksh[rows, :] = s
                u = s * v_buf[rows, cols].astype(f32)
                g = ga_buf[rows, cols].astype(f32) * q_buf[rows, cols].astype(f32)
                r = _dot(fw, jnp.concatenate([u, g], axis=1).astype(bf16), NN)
                scatter(uf, r[:, 0:w])
                scatter(gf, r[:, w:2 * w])
                kprev = kf[BL - 8:BL]
            return kprev
        lax.fori_loop(0, NB // tb, body, jnp.zeros((8, w), f32))

    def conv_freq(w, uf, gf, hf, zp, fg, pins):
        sgn = jnp.where(lax.broadcasted_iota(jnp.int32, (8, w), 0) % 2 == 0, 1.0, -1.0)
        total = 3 * (NB * (NB + 1) // 2)
        cnt = [0]
        uf, gf, hf = [r.at[_ds(fg * NB * 16, NB * 16, NB * 16), :] for r in (uf, gf, hf)]
        zp = [r.at[_ds(fg * 8, NB * BL - BL + 8, 8), :] for r in zp]

        def ld(ref, m):
            x = ref[m * 16:m * 16 + 16, :]
            return x[0:8], x[8:16]

        def chain(terms, conj):
            ar = ai = None
            for (a_, m, b_, n) in terms:
                hr, hi = ld(a_, m)
                gr, gi = ld(b_, n)
                k = cnt[0]
                cnt[0] += 1
                if ar is None:
                    pin = pins.at(k, total)
                    hr, hi = pinned(hr, pin), pinned(hi, pin)
                elif k % 3 == 0:
                    pin = pins.at(k, total)
                    ar, ai = pinned(ar, pin), pinned(ai, pin)
                if conj:
                    tr = hr * gr + hi * gi
                    ti = hr * gi - hi * gr
                else:
                    tr = hr * gr - hi * gi
                    ti = hr * gi + hi * gr
                ar = tr if ar is None else ar + tr
                ai = ti if ai is None else ai + ti
            return ar, ai

        def put(t, i, re, im):
            zp[t][i * BL:i * BL + 8, :] = _pk(jnp.concatenate([re, im], axis=0).astype(bf16))

        pz = pe = pc = None
        for i in range(NB):
            j = NB - 1 - i
            z = chain([(hf, m, uf, i - m) for m in range(i + 1)], False)
            put(0, i, *(z if pz is None else (z[0] - sgn * pz[1], z[1] + sgn * pz[0])))
            pz = z
            e = chain([(hf, m, gf, j + m) for m in range(NB - j)], True)
            put(1, j, *(e if pe is None else (e[0] + sgn * pe[1], e[1] - sgn * pe[0])))
            pe = e
            c = chain([(uf, m, gf, j + m) for m in range(NB - j)], True)
            put(2, j, *(c if pc is None else (c[0] + sgn * pc[1], c[1] - sgn * pc[0])))
            pc = c

    def conv_inv(c0, w, zp, ksh, tb, extra=None):
        cols = slice(c0, c0 + w)
        wj = [skt[j:j + 1, cols] for j in range(KS)]
        dvec = drow[:, cols]
        mi = 32

        def body(it, carry):
            dnext = carry[0]
            acc = list(carry[1:])
            b = NB // tb - 1 - it
            iv = iv_ref[...]
            dh = {}
            pin = None
            for i in reversed(range(tb)):
                blk = b * tb + i
                rows = _ds(blk * BL, BL, BL)
                zz = jnp.concatenate([_up(zp[t][rows, :]) for t in range(3)], axis=1)
                rs = []
                for k in range(BL // mi):
                    rs.append(_dot(pinned(iv[k * mi:(k + 1) * mi], pin), zz, NN))
                    if extra is not None:
                        pin = _up(extra(it, tb - 1 - i, k))
                r = jnp.concatenate(rs, axis=0)
                dh[i] = r[:, 2 * w:3 * w]
                if i % 2 == 0:
                    both = jnp.concatenate([dh[i], dh[i + 1]], axis=0)
                    h_buf[cols, _ds(blk * BL, 2 * BL, 2 * BL)] = both.astype(bf16).T
                s = ksh[rows, :]
                vv = v_buf[rows, cols].astype(f32)
                qv = q_buf[rows, cols].astype(f32)
                ga = ga_buf[rows, cols].astype(f32)
                kf = k_buf[rows, cols].astype(f32)
                u = s * vv
                g = ga * qv
                y = r[:, 0:w] + u * dvec
                ga_buf[rows, cols] = (qv * y).astype(bf16)
                q_buf[rows, cols] = (ga * y).astype(bf16)
                dkv = g * dvec + r[:, w:2 * w]
                v_buf[rows, cols] = (dkv * s).astype(bf16)
                dks = dkv * vv
                dp = jnp.concatenate([dks, dnext], axis=0)
                dk = None
                for j in range(KS):
                    sh = dks if j == 0 else pltpu.roll(dp, BL + 8 - j, 0)[0:BL]
                    dk = sh * wj[j] if dk is None else dk + sh * wj[j]
                    acc[j] = acc[j] + jnp.sum((sh * kf).reshape(BL // 8, 8, w), axis=0)
                k_buf[rows, cols] = dk.astype(bf16)
                acc[KS] = acc[KS] + jnp.sum((g * u).reshape(BL // 8, 8, w), axis=0)
                dnext = dks[0:8]
            for c in conv_out(c0, w, pl.multiple_of(b * tb * BL, tb * BL), tb * BL):
                c.start()
            return (dnext, *acc)
        out = lax.fori_loop(0, NB // tb, body, tuple(jnp.zeros((8, w), f32) for _ in range(KS + 2)))
        for j in range(KS + 1):
            red[j:j + 1, cols] = jnp.sum(out[1 + j], axis=0, keepdims=True)

    TB1, TB2 = 8, 4

    def conv_scratch(w):
        return ([pltpu.VMEM((NB * 2 * BL, w), f32)] * 3 + [pltpu.VMEM((NB * BL, w), u32)] * 3
                + [pltpu.VMEM((S, w), f32)])

    def cast(n, cbs, pin=None):
        j = (n % 4) * (H // 4) + n // 4
        row8 = lax.broadcasted_iota(jnp.int32, (8, 256), 0)
        src = res.at[_ds(j * 4 * R, 4 * R, 8), :]
        dst = dg.at[_ds(j * 40, 7 * 2 * D + 40, 8), :]
        for cb in cbs:
            w = src[:, cb * 256:(cb + 1) * 256]
            if pin is not None:
                w = jnp.concatenate([pinned(w[8 * k:8 * k + 8], pin if k in (0, 2, 5, 8, 11) else None)
                                     for k in range(12)], axis=0)
            parts = []
            for p in range(2):
                ev = w[2 * p * R:(2 * p + 1) * R]
                od = pltpu.roll(w[(2 * p + 1) * R:(2 * p + 2) * R], 4, 0)
                parts += [ev[0:16], jnp.where(row8 < 4, ev[16:24], od[0:8]), od[8:24]]
            dst[cb * 2 * D:cb * 2 * D + 40, :] = _pk(jnp.concatenate(parts, axis=0).astype(bf16))

    def front(ta):
        def phase1(wt, uf, gf, hf, z0, z1, z2, ksh):
            zp = (z0, z1, z2)

            def w_xpose(lo, hi):
                for j in range(lo, hi):
                    wt[j * 64:(j + 1) * 64, :] = _pk(w_buf[:, j * 128:(j + 1) * 128].T)
            cp_w.wait()
            w_xpose(0, 2 * D // 128)
            for c in cp_small:
                c.wait()
            skt[0:KS, 0:D] = sk_ref[...].astype(f32)
            drow[:, 0:D] = ssmd_ref[...].astype(f32).reshape(1, D)
            amax[...] = jnp.zeros_like(amax)
            conv_fwd(0, W1, uf, gf, hf, ksh, 4, True)
            row = lax.broadcasted_iota(jnp.int32, (R, TQ), 0)

            def proj(part, sb):
                w = _up(wt[_ds(part * (D // 2), D // 2, 8), :])
                xb = xg_buf[_ds(sb * TQ + jnp.where(part == 3, S, 0), TQ, TQ), :]
                r = _dot(w, xb, NT)
                m = jnp.max(jnp.abs(r).reshape(D // 8, 8, TQ), axis=0)
                amax[_ds(part * 8, 8, 8), :] = jnp.maximum(amax[_ds(part * 8, 8, 8), :], m)
                fill = jnp.where((part == 1) | (part == 2), 1.0, 0.0)
                dst = ta.at[_ds(part * HP, HP, 8), _ds(sb * TQ, TQ, TQ)]
                for h in range(H):
                    a = 8 * ((DH * h) // 8)
                    win = r[a:a + R]
                    if h % 2:
                        win = pltpu.roll(win, R - 4, 0)
                    dst[h * R:(h + 1) * R, :] = jnp.where(row >= DH, fill, win)
                return r

            def proj2(i, c):
                @pl.when(i < NQ)
                def _():
                    x_in(i).wait()

                @pl.when(i == NQ)
                def _():
                    for c_ in cp_mid:
                        c_.wait()
                    w_xpose(2 * D // 128, 3 * D // 128)
                    wt[3 * D // 2:2 * D, :] = _pk(wo_buf[...])
                pins = _Pins()
                for j in range(2):
                    pins.add(proj(2 * (i // NQ) + j, i % NQ), TQ // 128)
                xt[:, _ds(i * 256, 256, 256)] = _pk(xg_buf[_ds(i * 256, 256, 256), :].T)
                n = len(pins.items)
                for j in range(2):
                    conv_freq(W1, uf, gf, hf, zp, 2 * i + j, pins.window(j * n // 2 - 8, (j + 1) * n // 2 - 8))
                return c
            lax.fori_loop(0, 2 * NQ, proj2, 0)
            conv_inv(0, W1, zp, ksh, TB1)

        pl.run_scoped(phase1, pltpu.VMEM((2 * D, D), u32), *conv_scratch(W1))

        def key_major(t, h, cols, pin=None):
            blk = pinned(ta[_ds(t * HP + h * R, R, 8), cols], pin)
            return _pk(jnp.concatenate([blk, jnp.ones((8, CK), f32)], axis=0).astype(bf16).T)

        def q_weights(q):
            return _pk(jnp.concatenate([q * QS, jnp.zeros((8, TQ), f32)], axis=0).astype(bf16))

        def bwd_operands(o, do, inv):
            dop = (do * inv).astype(bf16).astype(f32)
            t = dop * o
            nd = (0.0 - t[0:8]) - t[8:16] - t[16:24]
            return dop, _pk(jnp.concatenate([dop, nd], axis=0).astype(bf16))

        def attn_fast(p0, p1, wq0, wq1, wdo0, wdo1, dop0, dop1, acco_buf, accq_buf, ds_buf,
                      kcur, vcur, tab):
            p_buf = (p0, p1)
            wq_buf = (wq0, wq1)
            wdo_buf = (wdo0, wdo1)
            dop_buf = (dop0, dop1)

            def half(c):
                return slice(c * CK // 2, (c + 1) * CK // 2)

            def full(c):
                return slice(c * CK, (c + 1) * CK)

            def tab_job(h, k, d, pin):
                src = ta.at[_ds(HP + h * R, R, 8), :]
                row = pinned(jnp.broadcast_to(src[d:d + 1, full(k)], (8, CK)) * QS, pin)
                tab[8 * k:8 * k + 8, d] = _tile(row, CK // 8, 1).T.reshape(8, 16, 128)

            def emit(s_lo, s_hi, hbase, lo, hi, vpu_lo, drain):
                st = {}

                def ok(g):
                    return lo <= g < hi

                def get(name, buf):
                    if name not in st:
                        st[name] = buf[...]
                    return st[name]

                def hrows(t, u):
                    return _ds(t * HP + (hbase + u // NQ) * R, R, 8)

                def qcols(u):
                    return slice((u % NQ) * TQ, (u % NQ + 1) * TQ)

                def accum(t, u, c, val, last_scale):
                    if u % NQ:
                        val = res[hrows(t, u), full(c)] + val
                    if u % NQ == NQ - 1 and last_scale is not None:
                        val = val * last_scale
                    res[hrows(t, u), full(c)] = val

                def mm(a, b, dims):
                    t = _dot(a, b, dims)
                    st['pins'].add(t)
                    return t

                def st_dp(s):
                    if ok(s):
                        u, c = divmod(s, NC)
                        dp = mm(_up(vcur[half(c), :]), _up(wdo_buf[u % 2][...]), NN)
                        st['ds_new'] = (_up(p_buf[u % 2][half(c), :]).astype(f32) * dp).astype(bf16)

                def st_dq(s):
                    if ok(s - 1):
                        u, c = divmod(s - 1, NC)
                        dsp = st['ds'] if 'ds' in st else _up(ds_buf[...])
                        t = mm(ta[hrows(1, u), full(c)], dsp, NN)
                        st['accq'] = t if c == 0 else get('accq', accq_buf) + t
                        if c == NC - 1:
                            res[hrows(1, u), qcols(u)] = st['accq'] * SCALE

                def st_dk(s):
                    if ok(s - 1):
                        u, c = divmod(s - 1, NC)
                        dsp = st['ds'] if 'ds' in st else _up(ds_buf[...])
                        accum(2, u, c, mm(ta[hrows(0, u), qcols(u)], dsp, NT), SCALE)

                def st_s(s):
                    if ok(s + OFF_A):
                        u, c = divmod(s + OFF_A, NC)
                        if c == 0:
                            wq_buf[u % 2][...] = q_weights(ta[hrows(0, u), qcols(u)])
                        spans = [slice(MGRP[c][0] * 8, (MGRP[c][-1] + 1) * 8)]
                        if s + OFF_A < vpu_lo:
                            spans.append(slice(VPASS[c][0] // 2 * 8, (VPASS[c][-1] // 2 + 1) * 8))
                        lhs = jnp.concatenate([kcur[sp, :] for sp in spans], axis=0)
                        p = _pk(jnp.exp2(mm(_up(lhs), _up(wq_buf[u % 2][...]), NN)).astype(bf16))
                        o = 0
                        for sp in spans:
                            p_buf[u % 2][sp, :] = p[o:o + sp.stop - sp.start]
                            o += sp.stop - sp.start

                def st_dv(s):
                    if ok(s):
                        u, c = divmod(s, NC)
                        accum(3, u, c, mm(dop_buf[u % 2][...], _up(p_buf[u % 2][half(c), :]), NT), None)

                def st_o(s):
                    if ok(s + OFF_O):
                        u, c = divmod(s + OFF_O, NC)
                        t = mm(ta[hrows(2, u), full(ORDER[c])], _up(p_buf[u % 2][half(ORDER[c]), :]), NN)
                        st['acco'] = t if c == 0 else get('acco', acco_buf) + t
                        if c == NC - 1:
                            acco = st['acco']
                            l = jnp.broadcast_to(acco[DH:DH + 1], (8, TQ))
                            r = pl.reciprocal(l, approx=True)
                            inv = _tile(r * (2.0 - l * r), 3, 1)
                            o = acco * inv
                            res[hrows(0, u), qcols(u)] = o
                            dop_buf[u % 2][...], wdo_buf[u % 2][...] = bwd_operands(
                                o, ta[hrows(3, u), qcols(u)], inv)

                def st_vpu(s, pins):
                    g = s + OFF_A + VL
                    if not (ok(g) and g >= vpu_lo):
                        return
                    u, c = divmod(g, NC)
                    if st.get('qb_u') != u:
                        qsrc = [ta.at[hrows(0, u), _ds((u % NQ) * TQ + l * 128, 128, 128)] for l in range(TQ // 128)]
                        st['qb_u'] = u
                        st['qb'] = jnp.concatenate([jnp.concatenate(
                            [jnp.broadcast_to(q[d:d + 1, :], (16, 128)) for q in qsrc], axis=1)[None]
                            for d in range(DH)], axis=0)
                    pt = 4
                    k = 0
                    for p in [VPASS[c][i] for i in (0, 3, 1, 2)]:
                        grp, lg = divmod(p, 2)
                        kb = tab[grp]
                        pr = jnp.concatenate([kb, kb], axis=2) * st['qb'][:, :, lg * 256:(lg + 1) * 256]
                        acc = pr[0]
                        for d in range(0, DH, pt):
                            pin = pins.at(k, len(VPASS[c]) * DH)
                            hp = (d // pt) % 2
                            acc = jnp.concatenate([pinned(acc[0:8], pin if hp == 0 else None),
                                                   pinned(acc[8:16], pin if hp == 1 else None)], axis=0)
                            k += min(pt, DH - d)
                            acc = jnp.sum(jnp.concatenate([acc[None], pr[max(d, 1):d + pt]], axis=0), axis=0)
                        p_buf[u % 2][grp * 8:(grp + 1) * 8, lg * 256:(lg + 1) * 256] = _pk(
                            jnp.exp2(acc).astype(bf16))

                def st_jobs(s, pins):
                    if drain and s_hi - 1 - NCS <= s < s_hi - 1:
                        e = s - (s_hi - 1 - NCS)
                        jl = range(e * NCE * 8 // NCS, (e + 1) * NCE * 8 // NCS)
                        for n, j in enumerate(jl):
                            cast(j // 8, [j % 8], pins.at(n, len(jl)))
                    u, c = divmod(s + OFF_A - LEAD, NC)
                    if u % NQ == NQ - 1 and ok((u + 1) * NC) and ok(u * NC) and ORDER[c] >= NVC:
                        kcur[half(ORDER[c]), :] = key_major(1, hbase + (u + 1) // NQ, full(ORDER[c]),
                                                            pins.at(0, 100))
                    hn, pos = divmod(s + OFF_A + VL + NC, NQ * NC)
                    p0 = pos - (_GDONE[7] + 1)
                    if 0 <= p0 < NTS and ok(hn * NQ * NC) and ok(hn * NQ * NC - 1):
                        jl = range(p0 * NVC * DH // NTS, (p0 + 1) * NVC * DH // NTS)
                        for n, j in enumerate(jl):
                            k = j // DH
                            assert _GDONE[8 * k + 7] < pos < NC + 8 * k * NC // NVG - 1
                            tab_job(hbase + hn, k, j % DH, pins.at((5 + 100 * n // len(jl)) % 100, 100))
                    u, c = divmod(s - 1, NC)
                    if u % NQ == NQ - 1 and ok((u + 1) * NC) and ok(u * NC):
                        vcur[half(c), :] = key_major(2, hbase + (u + 1) // NQ, full(c), pins.at(20, 100))

                for s in range(s_lo, s_hi):
                    st['pins'] = _Pins()
                    for fn in (st_dp, st_dq, st_dk, st_s, st_o, st_dv):
                        fn(s)
                    st_vpu(s, st['pins'])
                    st_jobs(s, st['pins'])
                    if 'ds_new' in st:
                        st['ds'] = st.pop('ds_new')
                if not drain:
                    ds_buf[...] = _pk(st['ds'])
                    accq_buf[...] = st['accq']
                    acco_buf[...] = st['acco']

            big = 1 << 30
            for c in range(NC):
                kcur[half(c), :] = key_major(1, 0, full(c))
                vcur[half(c), :] = key_major(2, 0, full(c))
            for j in range(NVC * DH):
                tab_job(0, j // DH, j % DH, None)
            emit(-OFF_A, S0, 0, 0, big, 1 + OFF_A, False)

            def body(it, c):
                emit(S0, S0 + NQ * NC, it, -big, big, -big, False)
                return c
            lax.fori_loop(0, NIT, body, 0)
            emit(S0, (H - NIT) * NQ * NC + 1, NIT, -big, (H - NIT) * NQ * NC, -big, True)
            flag[0] = NCE

        def attn_safe(s_buf, p_buf, wq_buf, wdo_buf, dop_buf, kcur, vcur):
            def unit(u, carry):
                h = u // NQ
                hr = [_ds(t * HP + h * R, R, 8) for t in range(4)]
                qc = _ds((u % NQ) * TQ, TQ, TQ)

                def rows(c):
                    return _ds(c * CK, CK, CK)

                def prows(c):
                    return _ds(c * (CK // 2), CK // 2, CK // 2)

                @pl.when(u % NQ == 0)
                def _():
                    def tr(c, z):
                        kcur[prows(c), :] = key_major(1, h, rows(c))
                        vcur[prows(c), :] = key_major(2, h, rows(c))
                        return z
                    lax.fori_loop(0, NC, tr, 0)

                wq_buf[...] = q_weights(ta[hr[0], qc])

                def scores(c, mx):
                    sc = _dot(_up(kcur[prows(c), :]), _up(wq_buf[...]), NN)
                    s_buf[rows(c), :] = sc
                    return jnp.maximum(mx, jnp.max(sc.reshape(CK // 8, 8, TQ), axis=0))
                mx = lax.fori_loop(0, NC, scores, jnp.full((8, TQ), -jnp.inf, f32))
                m = jnp.max(mx, axis=0, keepdims=True)

                def probs(c, acco):
                    p = jnp.exp2(s_buf[rows(c), :] - m).astype(bf16)
                    p_buf[prows(c), :] = _pk(p)
                    return acco + _dot(ta[hr[2], rows(c)], p, NN)
                acco = lax.fori_loop(0, NC, probs, jnp.zeros((R, TQ), f32))
                inv = 1.0 / acco[DH:DH + 1]
                o = acco * inv
                res[hr[0], qc] = o
                dop_buf[...], wdo_buf[...] = bwd_operands(o, ta[hr[3], qc], inv)

                def bwd(c, accq):
                    dp = _dot(_up(vcur[prows(c), :]), _up(wdo_buf[...]), NN)
                    pc = _up(p_buf[prows(c), :])
                    ds = (pc.astype(f32) * dp).astype(bf16)
                    for t, val in ((2, _dot(ta[hr[0], qc], ds, NT) * SCALE), (3, _dot(dop_buf[...], pc, NT))):
                        old = jnp.where(u % NQ == 0, 0.0, res[hr[t], rows(c)])
                        res[hr[t], rows(c)] = old + val
                    return accq + _dot(ta[hr[1], rows(c)], ds, NN)
                res[hr[1], qc] = lax.fori_loop(0, NC, bwd, jnp.zeros((R, TQ), f32)) * SCALE
                return carry
            lax.fori_loop(0, NU, unit, 0)

        def run_fast():
            pl.run_scoped(
                attn_fast,
                pltpu.VMEM((S // 2, TQ), u32), pltpu.VMEM((S // 2, TQ), u32),
                pltpu.VMEM((16, TQ), u32), pltpu.VMEM((16, TQ), u32),
                pltpu.VMEM((16, TQ), u32), pltpu.VMEM((16, TQ), u32),
                pltpu.VMEM((R, TQ), f32), pltpu.VMEM((R, TQ), f32),
                pltpu.VMEM((R, TQ), f32), pltpu.VMEM((R, TQ), f32), pltpu.VMEM((CK // 2, TQ), u32),
                pltpu.VMEM((S // 2, 32), u32), pltpu.VMEM((S // 2, 32), u32),
                pltpu.VMEM((NVG, DH, 16, 128), f32))

        def run_safe():
            pl.run_scoped(attn_safe, pltpu.VMEM((S, TQ), f32), pltpu.VMEM((S // 2, TQ), u32),
                          pltpu.VMEM((16, TQ), u32), pltpu.VMEM((16, TQ), u32), pltpu.VMEM((R, TQ), f32),
                          pltpu.VMEM((S // 2, 32), u32), pltpu.VMEM((S // 2, 32), u32))

        flag[0] = 0
        bound = (1.02 * DH * QS) * jnp.max(amax[0:8, :]) * jnp.max(amax[8:16, :])
        bounded = jnp.logical_and(bound <= SAFE, jnp.max(amax[16:32, :]) <= 1e20)
        pl.when(bounded)(run_fast)
        pl.when(jnp.logical_not(bounded))(run_safe)

    pl.run_scoped(front, pltpu.VMEM((4 * HP, S), f32))

    def phase2(on, dw_buf, uf, gf, hf, z0, z1, z2, ksh):
        zp = (z0, z1, z2)

        def cast_loop(n, c):
            cast(n, range(8))
            return c
        lax.fori_loop(flag[0], H, cast_loop, 0)
        for c in cp_c2:
            c.wait()
        conv_fwd(W1, W2, uf, gf, hf, ksh, 8, False)

        def dg_rows(ref, r0, n, cb0, cb1):
            return jnp.concatenate([ref[cb * 2 * D + r0:cb * 2 * D + r0 + n, :] for cb in range(cb0, cb1)], axis=1)

        def dx_out(i):
            rows = _ds(i * 256, 256, 256)
            return cp(xg_buf.at[rows, :], dx_hbm.at[rows, :], SEM_OUT)

        def dw_out(i):
            rows = _ds(i * 80, 80, 16)
            return cp(dw_buf.at[rows, :], dwqkv_hbm.at[rows, :], SEM_OUT)

        nob = 16
        tob = S // nob

        def ob_out(i):
            return cp(xg_buf.at[_ds(S + i * tob, tob, tob), :], out_hbm.at[_ds(i * tob, tob, tob), D:2 * D], SEM_OUT)

        def dxw(i, c):
            dgi = dg.at[_ds(i * 2 * D, 2 * D, 2 * D), :]
            md = 160
            pins = _Pins()
            outs = []
            for mb in range(D // md):
                acc = None
                for kk in range(8):
                    k0, k1 = kk * 256, min((kk + 1) * 256, 3 * D)
                    t = _dot(w_buf[mb * md:(mb + 1) * md, k0:k1], _up(dgi[D // 2 + k0 // 2:D // 2 + k1 // 2, :]), NN)
                    acc = t if acc is None else acc + t
                    pins.add(acc)
                outs.append(acc)
            xg_buf[_ds(i * 256, 256, 256), :] = jnp.concatenate(outs, axis=0).astype(bf16).T
            on[_ds(i * 128, 128, 128), :] = _pk(_up(dgi[0:D // 2, :]).T)
            lhs = xt.at[_ds(i * 40, 40, 8), :]
            dst = dw_buf.at[_ds(i * 80, 80, 16), :]
            for nb in range(3 * D // 128):
                acc = None
                for kk in range(4):
                    t = _dot(_up(lhs[:, kk * 512:(kk + 1) * 512]),
                             _up(dg_rows(dg, D // 2 + nb * 64, 64, 2 * kk, 2 * kk + 2)), NT)
                    acc = t if acc is None else acc + t
                    pins.add(acc)
                dst[:, nb * 128:(nb + 1) * 128] = acc.astype(bf16)
            n = len(pins.items)
            for j in range(2):
                conv_freq(W2, uf, gf, hf, zp, 2 * i + j, pins.window(j * n // 2 - 10, (j + 1) * n // 2 - 10))
            dx_out(i).start()
            dw_out(i).start()
            return c
        lax.fori_loop(0, 8, dxw, 0)

        wacc = [None] * 5

        def dwo_piece(it, kq, k):
            lhs = _up(dg_rows(dg.at[_ds(it * 80, 7 * 2 * D + 80, 8), :], 0, 80, 2 * kq, 2 * kq + 2))
            for nb in ((0,), (1,), (2,), (3, 4))[k]:
                t = _dot(lhs, xg_buf[S + kq * 512:S + (kq + 1) * 512, nb * 128:(nb + 1) * 128], NN)
                wacc[nb] = t if kq == 0 else wacc[nb] + t
            if kq == 3 and k == 3:
                dwo_buf[_ds(it * 160, 160, 16), :] = jnp.concatenate(wacc, axis=1).astype(bf16)
            return t[0:8]
        conv_inv(W1, W2, zp, ksh, TB2, dwo_piece)
        ssmd_ref[...] = red[KS:KS + 1, 0:D].reshape(D).astype(bf16)
        sk_ref[...] = red[0:KS, 0:D].astype(bf16)
        small_out = [cp(sk_ref, dsk_hbm, SEM_OUT), cp(ssmd_ref, dssmd_hbm, SEM_OUT), cp(dwo_buf, dwo_hbm, SEM_OUT)]
        for c in small_out:
            c.start()

        def outb(it, c):
            for j in range(nob // 2):
                i = it * (nob // 2) + j
                o = _up(on[_ds(i * (tob // 2), tob // 2, tob // 2), :])
                xg_buf[_ds(S + i * tob, tob, tob), :] = _dot(o, wo_buf[...], NN).astype(bf16)
                ob_out(i).start()
            return c
        lax.fori_loop(0, 2, outb, 0)

        for c in ([c for b in range(NB // TB1) for c in conv_out(0, W1, b * TB1 * BL, TB1 * BL)]
                  + [c for b in range(NB // TB2) for c in conv_out(W1, W2, b * TB2 * BL, TB2 * BL)]
                  + [dx_out(i) for i in range(8)] + [dw_out(i) for i in range(8)]
                  + small_out + [ob_out(i) for i in range(nob)]):
            c.wait()

    pl.run_scoped(phase2, pltpu.VMEM((S // 2, D), u32), pltpu.VMEM((D, 3 * D), bf16), *conv_scratch(W2))


@jax.jit
def pallas_concat_heads__ssm_conv_h3__softmax_full_mha__prompt_kernel(
    A_q: jax.Array,
    A_k: jax.Array,
    A_v: jax.Array,
    A_shift_k: jax.Array,
    A_ssm_k: jax.Array,
    A_ssm_D: jax.Array,
    B_x: jax.Array,
    B_wqkv: jax.Array,
    B_wo: jax.Array,
    grad_out: jax.Array,
):
    fw, iv = _dft_mats()
    fw = jnp.asarray(fw, dtype=bf16)
    iv = jnp.asarray(iv, dtype=bf16)
    zero = jnp.zeros((1,), jnp.int32)
    hbm = pl.BlockSpec(memory_space=pl.ANY)
    smem = pl.BlockSpec(memory_space=pltpu.SMEM)
    sd = jax.ShapeDtypeStruct
    outs = pl.pallas_call(
        _kernel,
        in_specs=[smem] + [hbm] * 12,
        out_specs=[hbm] * 10,
        out_shape=[sd((S, 2 * D), bf16), sd((S, D), bf16), sd((S, D), bf16), sd((S, D), bf16),
                   sd((KS, D), bf16), sd((D, S), bf16), sd((D,), bf16), sd((S, D), bf16),
                   sd((D, 3 * D), bf16), sd((D, D), bf16)],
        scratch_shapes=[
            pltpu.VMEM((8, 128 * 7), f32),
            pltpu.VMEM((S, D), bf16), pltpu.VMEM((S, D), bf16), pltpu.VMEM((S, D), bf16),
            pltpu.VMEM((S, D), bf16), pltpu.VMEM((D, S), bf16), pltpu.VMEM((2 * S, D), bf16),
            pltpu.VMEM((D, 3 * D), bf16), pltpu.VMEM((D, D), bf16), pltpu.VMEM((D, D), bf16),
            pltpu.VMEM((4 * HP, S), f32), pltpu.VMEM((D // 2, S), u32), pltpu.VMEM((8 * 2 * D, 256), u32),
            pltpu.VMEM((8, 1024), f32), pltpu.VMEM((32, TQ), f32),
            pltpu.VMEM((2 * BL, BL), bf16), pltpu.VMEM((BL, 2 * BL), bf16),
            pltpu.VMEM((1, 128 * 35), f32), pltpu.VMEM((KS, D), bf16), pltpu.VMEM((D,), bf16),
            pltpu.SMEM((1,), jnp.int32), pltpu.SemaphoreType.DMA((13,)),
        ],
        compiler_params=pltpu.CompilerParams(vmem_limit_bytes=124 * 1024 * 1024),
    )(zero, A_q.reshape(S, D), A_k.reshape(S, D), A_v.reshape(S, D), A_shift_k.T, A_ssm_k,
      A_ssm_D, B_x.reshape(S, D), B_wqkv, B_wo, grad_out.reshape(S, 2 * D), fw, iv)
    out, dq, dk, dv, dsk, dssmk, dssmd, dx, dwqkv, dwo = outs
    return (out.reshape(1, S, 2 * D), dq.reshape(1, S, D), dk.reshape(1, S, D), dv.reshape(1, S, D),
            dsk.T, dssmk, dssmd, dx.reshape(1, S, D), dwqkv, dwo)
```
